```python
import os as _os
_os.environ.setdefault('JAX_PLATFORMS', 'cpu')
import jax
import jax.numpy as jnp

def _softmax(x, axis=-1):
    return jax.nn.softmax(x, axis=axis)

def _gelu(x):
    return jax.nn.gelu(x, approximate=True)

def _silu(x):
    return jax.nn.silu(x)

def _sigmoid(x):
    return jax.nn.sigmoid(x)

def _layernorm(x, axis=-1, eps=1e-05):
    m = jnp.mean(x, axis=axis, keepdims=True)
    v = jnp.var(x, axis=axis, keepdims=True)
    return (x - m) / jnp.sqrt(v + eps)

def _scatter_add(tgt, idx, src, axis=0):
    return tgt.at[idx].add(src)

def _segment_sum(src, seg, n):
    return jax.ops.segment_sum(src, seg, n)

class _Rng:

    def __init__(self, key):
        self._k = key

    def _next(self):
        self._k, sub = jax.random.split(self._k)
        return sub

    def normal(self, shape):
        return jax.random.normal(self._next(), shape, dtype=jnp.bfloat16)

    def randint(self, lo, hi, shape):
        return jax.random.randint(self._next(), shape, lo, hi, dtype=jnp.int32)

    def uniform(self, shape, lo=0.0, hi=1.0):
        return jax.random.uniform(self._next(), shape, jnp.bfloat16, lo, hi)

    def permutation(self, n):
        return jax.random.permutation(self._next(), n)
kernel_name = 'adaLN_cond__grouped_kv_mqa__swiglu_ffn__prompt'

def setup_inputs():
    _rng = _Rng(jax.random.key(int.from_bytes(__import__("os").urandom(4), "little")))
    _w = lambda a: (lambda t: t.astype(jnp.bfloat16) if jnp.issubdtype(t.dtype, jnp.floating) else t)(jnp.asarray(a))

    def _A_setup():
        B, S, D, H = (1, 2048, 576, 32)
        Dh = D // H
        return {'x': _w((lambda *s: _rng.normal(s) * 0.05)(B, S, D)), 'wq': _w((lambda *s: _rng.normal(s) * 0.05)(D, H * Dh)), 'wk': _w((lambda *s: _rng.normal(s) * 0.05)(D, Dh)), 'wv': _w((lambda *s: _rng.normal(s) * 0.05)(D, Dh)), 'wo': _w((lambda *s: _rng.normal(s) * 0.05)(H * Dh, D))}
    _A_in = _A_setup()

    def _B_setup():
        B, S, D, F = (1, 2048, 576, 4608)
        return {'x': _w((lambda *s: _rng.normal(s) * 0.05)(B, S, D)), 'w_gate': _w((lambda *s: _rng.normal(s) * 0.05)(D, F)), 'w_up': _w((lambda *s: _rng.normal(s) * 0.05)(D, F)), 'w_down': _w((lambda *s: _rng.normal(s) * 0.05)(F, D))}
    _B_in = _B_setup()
    return {'A_x': _A_in['x'], 'A_wq': _A_in['wq'], 'A_wk': _A_in['wk'], 'A_wv': _A_in['wv'], 'A_wo': _A_in['wo'], 'B_x': _B_in['x'], 'B_w_gate': _B_in['w_gate'], 'B_w_up': _B_in['w_up'], 'B_w_down': _B_in['w_down'], 'c': _w((lambda *s: _rng.normal(s) * 0.05)(1, 576) * 8.0), 'w_mod': _w((lambda *s: _rng.normal(s) * 0.05)(576, 6 * 576) * 576 ** (-0.5) * 8.0)}

def reference(A_x, A_wq, A_wk, A_wv, A_wo, B_x, B_w_gate, B_w_up, B_w_down, c, w_mod):

    def _A_ref(x, wq, wk, wv, wo):
        B, S, D = x.shape
        H = 32
        Dh = D // H
        q = (lambda x, *d: x.transpose(*d))((x @ wq).reshape(B, S, H, Dh), 0, 2, 1, 3)
        k = x @ wk
        v = x @ wv
        scores = jnp.einsum('bhqd,bkd->bhqk', q, k) * Dh ** (-0.5)
        p = _softmax(scores, axis=-1)
        o = jnp.einsum('bhqk,bkd->bhqd', p, v)
        return (lambda x, *d: x.transpose(*d))(o, 0, 2, 1, 3).reshape(B, S, H * Dh) @ wo

    def _B_ref(x, w_gate, w_up, w_down):
        g = _silu(x @ w_gate)
        u = x @ w_up
        return g * u @ w_down
    x = A_x
    mod = (_silu(c) @ w_mod).reshape(c.shape[0], 6, 1, -1)
    sa, ca, ga, sb, cb, gb = (mod[:, 0].copy(), mod[:, 1].copy(), mod[:, 2].copy(), mod[:, 3].copy(), mod[:, 4].copy(), mod[:, 5].copy())
    h = _layernorm(x, axis=-1) * (1 + ca) + sa
    x = x + ga * _A_ref(h, A_wq, A_wk, A_wv, A_wo)
    h = _layernorm(x, axis=-1) * (1 + cb) + sb
    x = x + gb * _B_ref(h, B_w_gate, B_w_up, B_w_down)
    return x
```

```python
import math

import jax
import jax.numpy as jnp
from jax import lax
import jax.experimental.pallas as pl
import jax.experimental.pallas.tpu as pltpu

BF = jnp.bfloat16
F32 = jnp.float32
LANES = 128
N_HEADS = 32
EPS = 1e-5


def _build(S, D, F, TB=512, FC=512, FM=512):
    H = N_HEADS
    DH = D // H
    NL = TB // LANES
    NB = S // TB
    NT = S // LANES
    KC = 128
    NC = S // KC
    VR = 24
    QSCALE = DH ** -0.5 * math.log2(math.e)
    DP = D + 2 * 32

    def ln_mod(x, scale1, shift):
        n = x.shape[1]
        mean = jnp.sum(x, axis=0, keepdims=True) * (1.0 / D)
        xc = x - mean
        var = jnp.sum(xc * xc, axis=0, keepdims=True) * (1.0 / D)
        y = xc * lax.rsqrt(var + EPS)
        return y * jnp.tile(scale1, (1, n // LANES)) + jnp.tile(shift, (1, n // LANES))

    def kernel(x_hbm, wq_hbm, wk_hbm, wv_hbm, wo_hbm, wg_hbm, wu_hbm, wd_hbm, c_hbm, wm_hbm,
               out_hbm,
               x_v, wq_v, wk_v, wv_v, wo_v, wg_v, wu_v, wd_v, c_v, wm_v,
               wp_v, wot_v, mod_v, q_v, k_v, vt_v, s_v, o_v, x2_v, h2_v, acc_v, out_v,
               sem_x, sem_w, sem_o):
        def xcopy(b):
            return pltpu.make_async_copy(x_hbm.at[:, pl.ds(b * TB, TB)], x_v.at[:, pl.ds(b * TB, TB)], sem_x.at[b])

        cp_c = pltpu.make_async_copy(c_hbm, c_v, sem_w.at[0])
        cp_m0 = pltpu.make_async_copy(wm_hbm.at[:, pl.ds(0, 2 * D)], wm_v.at[:, pl.ds(0, 2 * D)], sem_w.at[1])
        cp_q = pltpu.make_async_copy(wq_hbm, wq_v, sem_w.at[2])
        cp_k = pltpu.make_async_copy(wk_hbm, wk_v, sem_w.at[3])
        cp_v = pltpu.make_async_copy(wv_hbm, wv_v, sem_w.at[4])
        cp_m1 = pltpu.make_async_copy(wm_hbm.at[:, pl.ds(2 * D, 4 * D)], wm_v.at[:, pl.ds(2 * D, 4 * D)], sem_w.at[5])
        cp_o = pltpu.make_async_copy(wo_hbm, wo_v, sem_w.at[6])
        cp_g = pltpu.make_async_copy(wg_hbm, wg_v, sem_w.at[7])
        cp_u = pltpu.make_async_copy(wu_hbm, wu_v, sem_w.at[8])
        cp_d = pltpu.make_async_copy(wd_hbm, wd_v, sem_w.at[9])

        cp_c.start()
        cp_q.start()
        cp_k.start()
        cp_v.start()
        cp_m0.start()
        for b in range(NB):
            xcopy(b).start()

        def mod_cols(sc, lo, hi):
            m = jnp.dot(sc, wm_v[:, lo:hi], preferred_element_type=F32)
            mod_v[lo:hi, :] = jnp.tile(m, (LANES // 8, 1)).T

        cp_q.wait()
        wp_v[0:D, :] = wq_v[...].astype(F32).T.astype(BF)
        cp_k.wait()
        cp_v.wait()
        z = jnp.zeros((32 - DH, D), F32)
        wp_v[D:DP, :] = jnp.concatenate([wk_v[...].astype(F32), z, wv_v[...].astype(F32), z], axis=0).astype(BF)
        cp_c.wait()
        cc = c_v[...].astype(F32)
        sc = jnp.broadcast_to(cc * jax.nn.sigmoid(cc), (8, D))
        cp_m0.wait()
        mod_cols(sc, 0, 2 * D)
        mod_v[D:2 * D, :] = mod_v[D:2 * D, :] + 1.0

        row = lax.broadcasted_iota(jnp.int32, (VR, TB), 0)
        for b in range(NB):
            xcopy(b).wait()
            if b == NB - 1:
                cp_m1.start()
                cp_o.start()
                cp_g.start()
                cp_u.start()
                cp_d.start()
            h = ln_mod(x_v[:, b * TB:(b + 1) * TB].astype(F32), mod_v[D:2 * D, :], mod_v[0:D, :])
            r = jnp.dot(wp_v[...], h.astype(BF), preferred_element_type=F32)
            for l in range(NL):
                t = b * NL + l
                q_v[t, 0:D, :] = r[0:D, l * LANES:(l + 1) * LANES] * QSCALE
                q_v[t, D:D + 8, :] = jnp.zeros((8, LANES), F32)
                kt = jnp.concatenate([r[D:D + 32, l * LANES:(l + 1) * LANES], jnp.zeros((LANES - 32, LANES), F32)], axis=0)
                k_v[t * LANES:(t + 1) * LANES, :] = kt.T
            vt_v[:, b * TB:(b + 1) * TB] = jnp.where(row == DH, 1.0, r[D + 32:D + 32 + VR, :])

        def load_q(u):
            b = u // H
            h = u % H
            return jnp.concatenate([q_v[b * NL + l, pl.ds(h * DH, VR), :] for l in range(NL)], axis=1)

        def colmax(s):
            m = s[0:8]
            for r in range(1, s.shape[0] // 8):
                m = jnp.maximum(m, s[8 * r:8 * r + 8])
            return m

        def fin(m8):
            return jnp.broadcast_to(jnp.max(m8, axis=0, keepdims=True), (8, TB))

        def qk(c, q):
            s = jnp.dot(k_v[c * KC:(c + 1) * KC, 0:VR], q, preferred_element_type=F32)
            s_v[c * KC:(c + 1) * KC, :] = s
            return colmax(s)

        def step(u, m, do_qk=True):
            mn = None
            acc = None
            if do_qk:
                q = load_q(u + 1)
            for c in range(NC):
                p = jnp.exp2(s_v[c * KC:(c + 1) * KC, :] - jnp.tile(m, (KC // 8, 1)))
                if do_qk:
                    t = qk(c, q)
                    mn = t if mn is None else jnp.maximum(mn, t)
                a = jnp.dot(vt_v[:, c * KC:(c + 1) * KC], p if do_qk else p.astype(BF), preferred_element_type=F32)
                acc = a if acc is None else acc + a
            o = acc * (1.0 / acc[DH:DH + 1, :])
            b = u // H
            h = u % H
            for l in range(NL):
                o_v[b * NL + l, pl.ds(h * DH, VR), :] = o[:, l * LANES:(l + 1) * LANES]
            return fin(mn) if do_qk else None

        q0 = load_q(0)
        mn = None
        for c in range(NC):
            t = qk(c, q0)
            mn = t if mn is None else jnp.maximum(mn, t)
        m = lax.fori_loop(0, NB * H - 1, step, fin(mn))
        step(NB * H - 1, m, do_qk=False)

        cp_m1.wait()
        mod_cols(sc, 2 * D, 6 * D)
        mod_v[4 * D:5 * D, :] = mod_v[4 * D:5 * D, :] + 1.0
        cp_o.wait()
        wot_v[...] = wo_v[...].astype(F32).T.astype(BF)
        for b in range(NB):
            o = jnp.concatenate([o_v[b * NL + l, 0:D, :] for l in range(NL)], axis=1)
            a = jnp.dot(wot_v[...], o.astype(BF), preferred_element_type=F32)
            x2 = x_v[:, b * TB:(b + 1) * TB].astype(F32) + jnp.tile(mod_v[2 * D:3 * D, :], (1, NL)) * a
            x2_v[:, b * TB:(b + 1) * TB] = x2
            h2 = ln_mod(x2, mod_v[4 * D:5 * D, :], mod_v[3 * D:4 * D, :])
            h2_v[b * TB:(b + 1) * TB, :] = h2.T.astype(BF)

        cp_g.wait()
        cp_u.wait()
        cp_d.wait()

        def ocopy(b):
            return pltpu.make_async_copy(out_v.at[:, pl.ds(b * FM, FM)], out_hbm.at[:, pl.ds(b * FM, FM)], sem_o.at[b])

        def ffn(b, _):
            r0 = pl.multiple_of(b * FM, FM)
            h2 = h2_v[pl.ds(r0, FM), :]
            acc = None
            for f in range(F // FC):
                g = jnp.dot(h2, wg_v[:, f * FC:(f + 1) * FC], preferred_element_type=F32)
                u = jnp.dot(h2, wu_v[:, f * FC:(f + 1) * FC], preferred_element_type=F32)
                t = 0.5 * g
                act = ((t + t * jnp.tanh(t)) * u).astype(BF)
                d = lax.dot_general(wd_v[:, f * FC:(f + 1) * FC], act, (((1,), (1,)), ((), ())),
                                    preferred_element_type=F32)
                acc = d if acc is None else acc + d
            y = x2_v[:, pl.ds(r0, FM)] + jnp.tile(mod_v[5 * D:6 * D, :], (1, FM // LANES)) * acc
            out_v[:, pl.ds(r0, FM)] = y.astype(BF)
            ocopy(b).start()

        lax.fori_loop(0, S // FM, ffn, None)
        for b in range(S // FM):
            ocopy(b).wait()

    scratch = [
        pltpu.VMEM((D, S), BF), pltpu.VMEM((D, D), BF), pltpu.VMEM((DH, D), BF), pltpu.VMEM((DH, D), BF),
        pltpu.VMEM((D, D), BF), pltpu.VMEM((D, F), BF), pltpu.VMEM((D, F), BF), pltpu.VMEM((D, F), BF),
        pltpu.VMEM((1, D), BF), pltpu.VMEM((D, 6 * D), BF),
        pltpu.VMEM((DP, D), BF), pltpu.VMEM((D, D), BF), pltpu.VMEM((6 * D, LANES), F32),
        pltpu.VMEM((NT, D + 8, LANES), F32), pltpu.VMEM((S, LANES), F32), pltpu.VMEM((VR, S), F32),
        pltpu.VMEM((S, TB), F32), pltpu.VMEM((NT, D + 8, LANES), F32), pltpu.VMEM((D, S), F32),
        pltpu.VMEM((S, D), BF), pltpu.VMEM((D, FM), F32), pltpu.VMEM((D, S), BF),
        pltpu.SemaphoreType.DMA((NB,)), pltpu.SemaphoreType.DMA((10,)), pltpu.SemaphoreType.DMA((S // FM,)),
    ]
    return pl.pallas_call(
        kernel,
        out_shape=jax.ShapeDtypeStruct((D, S), BF),
        in_specs=[pl.BlockSpec(memory_space=pl.ANY)] * 10,
        out_specs=pl.BlockSpec(memory_space=pl.ANY),
        scratch_shapes=scratch,
        compiler_params=pltpu.CompilerParams(vmem_limit_bytes=110 * 2 ** 20),
        name="adaln_mqa_swiglu",
    )


def make(**cfg):
    @jax.jit
    def pallas_adaLN_cond__grouped_kv_mqa__swiglu_ffn__prompt_kernel(
            A_x, A_wq, A_wk, A_wv, A_wo, B_x, B_w_gate, B_w_up, B_w_down, c, w_mod):
        del B_x
        _, S, D = A_x.shape
        F = B_w_gate.shape[1]
        out_t = _build(S, D, F, **cfg)(A_x[0].T, A_wq, A_wk.T, A_wv.T, A_wo, B_w_gate, B_w_up, B_w_down.T, c, w_mod)
        return out_t.T[None]
    return pallas_adaLN_cond__grouped_kv_mqa__swiglu_ffn__prompt_kernel


pallas_adaLN_cond__grouped_kv_mqa__swiglu_ffn__prompt_kernel = make()
```

```python
import math

import jax
import jax.numpy as jnp
from jax import lax
import jax.experimental.pallas as pl
import jax.experimental.pallas.tpu as pltpu

BF = jnp.bfloat16
F32 = jnp.float32
LANES = 128
SUB = 8
N_HEADS = 32
EPS = 1e-5
ROW_SUM_MIN = 2.0 ** -30
ROW_SUM_MAX = 2.0 ** 100

_STRASSEN = (
    (((1, 1, 1), (1, 0, 0)), ((1, 1, 1), (1, 0, 0)), ((1, 0, 0), (1, 1, 1))),
    (((1, 1, 0), (1, 1, 1)), ((1, 0, 0),), ((1, 1, 0), (-1, 1, 1))),
    (((1, 0, 0),), ((1, 0, 1), (-1, 1, 1)), ((1, 0, 1), (1, 1, 1))),
    (((1, 1, 1),), ((1, 1, 0), (-1, 0, 0)), ((1, 0, 0), (1, 1, 0))),
    (((1, 0, 1), (1, 0, 0)), ((1, 1, 1),), ((-1, 0, 0), (1, 0, 1))),
    (((1, 1, 0), (-1, 0, 0)), ((1, 0, 0), (1, 0, 1)), ((1, 1, 1),)),
    (((1, 0, 1), (-1, 1, 1)), ((1, 1, 0), (1, 1, 1)), ((1, 0, 0),)),
)
_ORDER = (1, 0, 3, 4, 6, 2, 5)
_INNER_ORDER = (1, 3, 4, 2, 0, 6, 5)


def _strassen(prod, mirror=False, order=_ORDER):
    c = {}
    for j in order:
        a, b, outs = _STRASSEN[j]
        m = prod(j, a, tuple((s, k, n ^ mirror) for s, k, n in b))
        for s, r, n in outs:
            key = r, n ^ mirror
            c[key] = (1, _signed_sum([(s, m), c[key]])) if key in c else (s, m)
    return [[c[r, n][1] for n in range(2)] for r in range(2)]


def _strassen_wide(prod):
    x1 = prod(((1, 0, 0), (1, 1, 1)), None, ((1, 0, 0), (1, 1, 1)), ())
    p4 = prod(((1, 1, 1),), ((1, 0, 0),), ((1, 1, 0), (-1, 0, 0)), ((1, 0, 0), (-1, 1, 0)))
    p5 = prod(((1, 0, 0), (1, 0, 1)), None, ((1, 1, 1),), ((-1, 1, 0),))
    c11 = prod(((1, 0, 1), (-1, 1, 1)), ((1, 0, 2),), ((1, 1, 0), (1, 1, 1)), ((1, 2, 0),)) + (p4 - p5 + x1)
    p2 = prod(((1, 1, 0), (1, 1, 1)), None, ((1, 0, 0),), ((-1, 0, 1),))
    p3 = prod(((1, 0, 0),), ((1, 1, 1),), ((1, 0, 1), (-1, 1, 1)), ((1, 1, 1), (-1, 0, 1)))
    c22 = prod(((1, 1, 0), (-1, 0, 0)), ((1, 1, 2),), ((1, 0, 0), (1, 0, 1)), ((1, 2, 1),)) + (p3 + (x1 - p2))
    y1 = prod(((1, 0, 0), (1, 1, 1)), None, (), ((1, 0, 1), (1, 1, 0)))
    c12 = prod(((1, 0, 2),), ((1, 0, 1), (-1, 1, 1)), ((1, 2, 1),), ((1, 1, 0), (1, 1, 1))) + (y1 + (p3 + p5))
    c21 = prod(((1, 1, 2),), ((1, 1, 0), (-1, 0, 0)), ((1, 2, 0),), ((1, 0, 0), (1, 0, 1))) + (y1 + (p2 + p4))
    return [[c11, c12], [c21, c22]]


def _left_sums(a11, a12, a21, a22):
    return a11 + a22, a21 + a22, a11, a22, a11 + a12, a21 - a11, a12 - a22


def _signed_sum(terms):
    (sign, out), *rest = sorted(terms, key=lambda t: -t[0])
    if rest or sign < 0:
        out = out.astype(F32) if sign > 0 else -out.astype(F32)
    for sign, t in rest:
        out = out + t.astype(F32) if sign > 0 else out - t.astype(F32)
    return out


def _block(c):
    return jnp.concatenate([jnp.concatenate(row, axis=1) for row in c], axis=0)


def _dot(a, b, trans_b=False):
    return lax.dot_general(a, b, (((1,), (1 if trans_b else 0,)), ((), ())), preferred_element_type=F32)


def _span(i, n):
    return slice(i * n, (i + 1) * n)


def _lane(l):
    return _span(l, LANES)


def _zeros_from(i):
    count = [0]

    def zero():
        count[0] += 1
        return (i + count[0]) >> 16

    return zero


def _shifted(x, n, rows):
    above, below = [[jnp.zeros((m, x.shape[1]), F32)] if m else [] for m in (n, rows - n - x.shape[0])]
    return jnp.concatenate(above + [x] + below, axis=0)


def _build(S, D, F):
    H = N_HEADS
    DH = D // H
    HH = DH // 2
    TB = 512
    NL = TB // LANES
    NB = S // TB
    HG = 4
    GR = HG * DH
    GB = H // HG
    VR = 24
    KC = LANES
    NC = S // KC
    G = KC // SUB
    NV = 3
    POS = ((15, 8, 3), (6, 12, 1))
    UNROLL = 2
    QSCALE = DH ** -0.5 * math.log2(math.e)
    DP = 2 * VR + D
    FW = 512
    NF = F // FW
    HB, HD, HF, QS = TB // 2, D // 2, FW // 2, S // 4
    K1 = 2 * LANES
    PACE = (0, 1, 2, 3, 4, 5, 6, 7, 8, 9, 14, 15, 16, 17, 18, 19)
    assert (D, DH) == (576, 18) and S % (2 * TB) == 0 and F % FW == 0 and 2 * NC <= 2 * F // LANES

    def norm(x, scale, shift):
        mean = jnp.sum(x, axis=0, keepdims=True) * (1.0 / D)
        xc = x - mean
        variance = jnp.sum(xc * xc, axis=0, keepdims=True) * (1.0 / D)
        return xc * lax.rsqrt(variance + EPS) * scale + shift

    def sum_row(j):
        return DH + 2 * j if DH + 2 * j < VR else 0

    def arrange(pos, groups):
        rows = dict(zip([g for g in reversed(range(G)) if g not in pos] + list(pos), groups))
        return jnp.concatenate([rows[g] for g in range(G)], axis=0)

    def kernel(x_hbm, wq_hbm, wk_hbm, wv_hbm, wo_hbm, wg_hbm, wu_hbm, wd_hbm, c_hbm, wm_hbm, out_hbm,
               act_v, q_v, t_v, o_v, p_v, pa_v, r_v, s0_v, s1_v, a_v, mod_v, x_v, wg_v, wu_v, wd_v,
               wq_v, wo_v, wm0_v, wm1_v, wp_v, wot_v, u_v, wk_v, wv_v, c_v, sem):
        s_v = (s0_v, s1_v)

        def ks_rows(n, d):
            return _span(n * HH + d, SUB)

        def kb_rows(d):
            return _span(7 * HH + d, SUB)

        def vt_rows(j, t):
            return pl.ds((7 * HH + DH) * SUB + (2 * j + t) * VR, VR)

        cp_c, cp_k, cp_v, cp_q, cp_o, cp_m0, cp_m1, *cp_x = [
            pltpu.make_async_copy(src, dst, sem.at[n]) for n, (src, dst) in enumerate(
                [(c_hbm, c_v), (wk_hbm, wk_v), (wv_hbm, wv_v), (wq_hbm, wq_v), (wo_hbm, wo_v),
                 (wm_hbm.at[:, pl.ds(0, 2 * D)], wm0_v), (wm_hbm.at[:, pl.ds(2 * D, 4 * D)], wm1_v)]
                + [(x_hbm.at[:, pl.ds(b * TB, TB)], x_v.at[b]) for b in range(NB)])]
        cp_w = [pltpu.make_async_copy(src.at[:, pl.ds(i * FW, FW)], dst.at[i], sem.at[7 + NB])
                for src, dst in ((wg_hbm, wg_v), (wu_hbm, wu_v), (wd_hbm, wd_v)) for i in range(NF)]

        def cp_out(b):
            return pltpu.make_async_copy(x_v.at[b], out_hbm.at[:, pl.ds(b * TB, TB)], sem.at[7 + b])

        def modulation(w, first):
            m = _dot(wp_v[DP:DP + SUB, :], w)
            mod_v[first:first + w.shape[1], :] = jnp.tile(m, (LANES // SUB, 1)).T

        for cp in [cp_m0, cp_c, cp_k, cp_v, cp_x[0], cp_q] + cp_x[1:]:
            cp.start()
        p_v[...] = jnp.zeros_like(p_v)
        pa_v[...] = jnp.zeros_like(pa_v)
        cp_m0.wait()
        cp_c.wait()
        cc = c_v[...].astype(F32)
        wp_v[DP:DP + SUB, :] = jnp.broadcast_to(cc * jax.nn.sigmoid(cc), (SUB, D))
        modulation(wm0_v[...], 0)
        mod_v[_span(1, D), :] += 1.0
        cp_k.wait()
        cp_v.wait()
        cp_x[0].wait()
        wp_v[0:2 * VR, :] = jnp.concatenate([_shifted(w[...].astype(F32), 0, VR) for w in (wk_v, wv_v)], axis=0)

        def norm1(b, l):
            return norm(x_v[b, :, _lane(l)].astype(F32), mod_v[_span(1, D), :], mod_v[_span(0, D), :])

        def put_kv(c, kt, vt):
            kk = jnp.concatenate([_shifted(kt, 2 * j, LANES // HG) for j in range(HG)], axis=0).T
            kk = jnp.concatenate(
                [kk[_span(g, SUB)] for g in list(reversed(range(G - NV))) + list(range(G - NV, G))], axis=0)
            row = lax.broadcasted_iota(jnp.int32, (VR, KC), 0)
            for t, pos in enumerate(POS):
                free = [g for g in range(G) if g not in pos]
                src = [G - NV + pos.index(g) if g in pos else free.index(g) for g in range(G)]
                cuts = [g for g in range(G) if g == 0 or src[g] != src[g - 1] + 1] + [G]
                v = jnp.concatenate([vt[:, src[a] * SUB:(src[a] + e - a) * SUB] for a, e in zip(cuts, cuts[1:])],
                                    axis=1)
                for j in range(HG):
                    act_v[c, vt_rows(j, t), :] = jnp.where(row == sum_row(j), 1.0, _shifted(v[:DH], 2 * j, VR))
            for j in range(HG):
                act_v[NC + c, _span(j, KC), 0:VR] = kk[:, j * (LANES // HG):j * (LANES // HG) + VR]

            def spread(g, d):
                return jnp.broadcast_to(kk[_span(g, SUB), d:d + 1], (SUB, LANES))

            for d in range(HH):
                a11, a12, a21, a22 = [spread(G - NV + g, d + k) for g in range(2) for k in (0, HH)]
                s1 = a21 + a22
                s2 = s1 - a11
                for n, a in enumerate((a11, a12, a12 - s2, a22, s1, s2, a11 - a21)):
                    act_v[c, ks_rows(n, d), :] = a
            for d in range(DH):
                act_v[c, kb_rows(d), :] = spread(G - 1, d)

        def put_q(b, l, left, right):
            low = lax.broadcasted_iota(jnp.int32, (GR, LANES), 0) % DH < HH
            for g in range(GB):
                qa, qb = left[_span(g, GR)], right[_span(g, GR)]
                t13 = qb - jnp.where(low, qa, _shifted(qb[:GR - HH], HH, GR))
                t2 = qb - _shifted(t13[:GR - HH], HH, GR)
                q_v[b * GB + g, :, _lane(l)] = qa
                q_v[b * GB + g, :, _lane(l + NL // 2)] = qb
                t_v[b * GB + g, :, _lane(l)] = t13
                t_v[b * GB + g, :, _lane(l + NL // 2)] = jnp.where(low, _shifted(t2[HH:], 0, GR), qa - t2)

        tiles = [(b, l + t) for b in range(NB) for l in range(NL // 2) for t in (0, NL // 2)]
        early = [norm1(*t) for t in tiles[:2]]
        cp_q.wait()
        wp_v[2 * VR:DP, :] = wq_v[...].T.astype(F32)
        prev = centre = left = None
        for n in range(len(tiles) + 1):
            if n < len(tiles):
                h = early[n] if n < len(early) else norm1(*tiles[n])
                r = _dot(wp_v[0:DP, 0:LANES], h[0:LANES])
                if n == NL - 1:
                    for cp in cp_x[1:]:
                        cp.wait()
                    for cp in [cp_m1, cp_o] + cp_w:
                        cp.start()
                r = _dot(wp_v[0:DP, LANES:D], h[LANES:D]) + r
            if n:
                b, l = tiles[n - 1]
                if n == 1:
                    centre = jnp.mean(prev[0:DH], axis=1, keepdims=True)
                put_kv(b * NL + l, prev[0:DH] - centre, prev[VR:2 * VR])
                if n % 2:
                    left = prev[2 * VR:] * QSCALE
                else:
                    put_q(b, l - NL // 2, left, prev[2 * VR:] * QSCALE)
            prev = r

        push_order = [(l + NL // 2) % NL for l in range(NL)]

        def finish(g):
            for l in push_order:
                o_v[g, HG - 1, :, _lane(l)] = (
                    _dot(act_v[NC - 1, vt_rows(HG - 1, l // (NL // 2)), :], p_v[:, _lane(l)]) + pa_v[:, _lane(l)])

        def attend_centred(i, _):
            zero = _zeros_from(i)

            def chain(keys, ref, g, row, l, acc=None):
                for d, k in enumerate(keys):
                    t = k * ref[g, pl.ds(row + d, 1), _lane(l)]
                    acc = t if acc is None else acc + t
                return acc

            def vector_scores(g, j, c):
                g = g + zero()
                ks = [[act_v[c, ks_rows(n, d), :] for d in range(HH)] for n in range(7)]
                kb = [act_v[c, kb_rows(d), :] for d in range(DH)]
                out = [None] * NL
                for la in range(NL // 2):
                    lb = la + NL // 2

                    def prod(n, acc=None):
                        ref, k, l = ((q_v, 0, la), (q_v, HH, la), (q_v, HH, lb),
                                     (t_v, HH, lb), (t_v, 0, la), (t_v, 0, lb), (t_v, HH, la))[n]
                        return chain(ks[n], ref, g, j * DH + k, l, acc)

                    p1 = prod(0)
                    c11 = prod(1, p1)
                    u2 = prod(5, p1)
                    u3 = prod(6, u2)
                    p5 = prod(4)
                    out[lb] = [prod(2, u2 + p5), u3 + p5]
                    out[la] = [c11, prod(3, u3)]
                g = g + zero()
                for l in range(NL):
                    lo, hi = [chain(kb[k:k + HH], q_v, g, j * DH + k, l) for k in (0, HH)]
                    out[l].append(lo + hi)
                return out

            steps = [(n, j, c) for n in range(UNROLL) for j in range(HG) for c in range(NC)]
            base = {(n, j): zero() for n in range(UNROLL) for j in range(HG)}
            prev = acc = None
            for step in steps + [None]:
                cur = None
                if step:
                    n, j, c = step
                    cur = step, jnp.exp2(_dot(act_v[base[n, j] + NC + c, j * KC:(j + 1) * KC - NV * SUB, 0:VR],
                                              q_v[i * UNROLL + n, 2 * SUB * j:2 * SUB * j + VR, :]))
                if prev:
                    (n, j, c), e = prev
                    g = i * UNROLL + n
                    chunk = base[n, j] + c
                    extra = vector_scores(g, j, chunk)
                    new = {}
                    for l in push_order:
                        t = l // (NL // 2)
                        p = arrange(POS[t], [e[_span(x, SUB), _lane(l)] for x in range(G - NV)]
                                    + [jnp.exp2(v) for v in extra[l]])
                        if step:
                            a = _dot(act_v[chunk, vt_rows(j, t), :], p)
                            new[l] = a + acc[l] if c else a
                        else:
                            p_v[:, _lane(l)] = p
                            pa_v[:, _lane(l)] = acc[l]
                    acc = new
                    if c == NC - 1:
                        for l in acc:
                            o_v[g, j, :, _lane(l)] = acc[l]
                else:
                    finish(jnp.maximum(i * UNROLL - 1, 0))
                prev = cur

        def attend_row_max(u, _):
            g, j = u // HG, u % HG
            q = q_v[g, pl.ds(pl.multiple_of(2 * SUB * j, SUB), VR), :]
            m = acc = None
            for c in range(NC):
                s = _dot(act_v[NC + c, pl.ds(pl.multiple_of(j * KC, KC), KC), 0:VR], q)
                s_v[c % 2][0, _span(c // 2, KC), :] = s
                t = jnp.max(s, axis=0, keepdims=True)
                m = jnp.maximum(m, t) if c else t
            for c in range(NC):
                p = jnp.exp2(s_v[c % 2][u >> 16, _span(c // 2, KC), :] - m)
                a = _dot(act_v[c, vt_rows(j, 0), :], arrange(POS[0], [p[_span(x, SUB)] for x in range(G)]))
                acc = a + acc if c else a
            o_v[g, j] = acc

        lax.fori_loop(0, NB * GB // UNROLL, attend_centred, None)

        def heads(b, l, checks):
            row = lax.broadcasted_iota(jnp.int32, (SUB, LANES), 0)
            for h0 in range(0, H, SUB):
                total = None
                for h in range(h0, h0 + SUB):
                    t = o_v[b * GB + h // HG, h % HG, pl.ds(sum_row(h % HG), 1), _lane(l)]
                    total = t if total is None else jnp.where(row == h - h0, t, total)
                checks.append((total >= ROW_SUM_MIN) & (total <= ROW_SUM_MAX))
                r_v[b, h0:h0 + SUB, _lane(l)] = 1.0 / total
            out = []
            for h in range(H):
                o = o_v[b * GB + h // HG, h % HG, :, _lane(l)] * r_v[b, pl.ds(h, 1), _lane(l)]
                top = jnp.where(row < 2 * (h % HG), out.pop(), o[:SUB]) if h % HG else o[:SUB]
                out += [top, o[SUB:2 * SUB], o[2 * SUB:]]
            return jnp.concatenate(out, axis=0)

        def project_out(b, l, checks):
            h2 = []
            for t in (l, l + NL // 2):
                o = heads(b, t, checks)
                attn = None
                for k in range(0, D, LANES):
                    a = _dot(wot_v[:, k:min(k + LANES, D)], o[k:k + LANES])
                    attn = a + attn if k else a
                checks.append(jnp.abs(attn[:SUB]) < jnp.inf)
                x2 = x_v[b, :, _lane(t)].astype(F32) + mod_v[_span(2, D), :] * attn
                t_v[_span(b, GB), :, _lane(t)] = x2.reshape(GB, GR, LANES)
                h = norm(x2, mod_v[_span(4, D), :], mod_v[_span(3, D), :])
                h2.append(jnp.concatenate([h, h[2 * K1:]], axis=0).T)
            rows = _span(b * (NL // 2) + l, LANES)
            for j, a in enumerate(_left_sums(*[h[:, k:k + K1] for h in h2 for k in (0, K1)])):
                a_v[j, rows, 0:K1] = a
            r1, r2 = [h[:, 2 * K1:] for h in h2]
            for j, a in ((0, r2), (3, r2), (4, r1), (6, r1 - r2)):
                a_v[j, rows, K1:] = a

        cp_m1.wait()
        cp_o.wait()
        finish(NB * GB - 1)
        wot_v[...] = wo_v[...].T.astype(F32)
        split = pl.cdiv(3 * D, LANES) * LANES
        modulation(wm1_v[:, :split], 2 * D)
        mod_v[_span(3, D), :] *= 0.5
        mod_v[_span(4, D), :] = 0.5 * mod_v[_span(4, D), :] + 0.5

        def attempt(state):
            @pl.when(state[0] == 1)
            def _():
                lax.fori_loop(0, NB * H, attend_row_max, None)

            modulation(wm1_v[:, split:], 2 * D + split)
            checks = []
            for b in range(NB):
                for l in range(NL // 2):
                    project_out(b, l, checks)
            good = jnp.ones((SUB, LANES), F32)
            for ok in checks:
                good = jnp.where(ok, good, 0.0)
            return state[0] + 1, jnp.min(good).astype(jnp.int32)

        lax.while_loop(lambda state: (state[0] < 2) & (state[1] == 0), attempt, (0, 0))

        def gate_up(i, _):
            zero = _zeros_from(i)
            passes = []

            def outer(j, a, b):
                rest = [t for t in b if t[1] == 1] if b[0][1] == 1 else []

                def left(z, terms):
                    return _signed_sum([(s, a_v[z, _span(m, QS), _lane(k)]) for s, m, k in terms])

                def right(terms, first, rows):
                    return _signed_sum([
                        (s * ss, (wg_v, wu_v)[n][i + zero(), pl.ds(k * K1 + kk * LANES + first * (kk < 2), rows),
                                                 _span(nn, HF)])
                        for ss, kk, nn in terms for s, k, n in (b if kk < 2 else rest)])

                def inner(jj, aa, bb):
                    lhs, rhs = left(j + zero(), aa), right(bb, 0, LANES)
                    if j == jj == _ORDER[-1]:
                        return jnp.concatenate([_dot(lhs[_span(m, QS // 2)], rhs) for m in range(2)], axis=0)
                    passes.append(_dot(lhs, rhs))
                    return passes[-1]

                def wide(a_low, a_high, b_low, b_high):
                    z = j + zero()
                    half = LANES // 2
                    lhs = left(z, a_low)
                    if a_high:
                        lhs = jnp.where(lax.broadcasted_iota(jnp.int32, lhs.shape, 1) < half, lhs, left(z, a_high))
                    rhs = [right(t, first, half).astype(F32) if t else jnp.zeros((half, HF), F32)
                           for t, first in ((b_low, 0), (b_high, half))]
                    passes.append(_dot(lhs, jnp.concatenate(rhs, axis=0)))
                    return passes[-1]

                return _block(_strassen_wide(wide) if rest else _strassen(inner, j == 5, _INNER_ORDER))

            for m, (t, up) in enumerate(_strassen(outer)):
                s_v[m][0] = t + t * jnp.tanh(t)
                act = s_v[m][zero()] * up
                for l in range(FW // LANES):
                    act_v[(m * NF + i) * (FW // LANES) + l, 0:S // 2, :] = act[:, _lane(l)]

            always = lax.broadcasted_iota(jnp.int32, (2 * SUB, HF), 0) >= zero()
            jobs = [(j, r) for j in range(7) for r in range(0, HD // 2, SUB)]
            slab = [i + zero() for _ in range(7)]
            for n, (j, r) in enumerate(jobs):
                w = _signed_sum([
                    (s, jnp.concatenate([wd_v[slab[j], pl.ds(m * HD + o + r, SUB), _span(k, HF)].astype(F32)
                                         for o in (0, HD // 2)], axis=0)) for s, m, k in _STRASSEN[j][0]])
                when, row = divmod(n * len(PACE) * (QS // SUB) // len(jobs), QS // SUB)
                w = jnp.where(always, w, jnp.tile(passes[2 * PACE[when] + 1][_span(row, SUB)], (2, 1)))
                sums = _left_sums(*[w[_span(m, SUB), _lane(k)] for m in range(2) for k in range(2)])
                u_v[i, j, r:r + SUB, :] = jnp.concatenate(sums, axis=1).astype(BF)

        def down(b, _):
            zero = _zeros_from(b)

            def outer(j, _, terms):
                def inner(jj, _, sub):
                    r0 = pl.multiple_of((b + zero()) * HB, HB)
                    acc = None
                    for i in range(NF):
                        rhs = _signed_sum([
                            (s * ss, act_v[(n * NF + i) * (FW // LANES) + 2 * k + kk, pl.ds(r0 + nn * LANES, LANES), :])
                            for ss, kk, nn in sub for s, k, n in terms])
                        lhs = u_v[i, j, :, _lane(jj)]
                        if j == jj == _ORDER[-1] and i == NF - 1:
                            r = jnp.concatenate([_dot(lhs[_span(m, HD // 6)], rhs.astype(BF), True)
                                                 for m in range(3)], axis=0)
                        else:
                            r = _dot(lhs, rhs.astype(BF), True)
                        acc = r + acc if i else r
                    return acc

                return _block(_strassen(inner, j in (1, 4, 5, 6), _INNER_ORDER))

            x2 = t_v[pl.ds(b * GB, GB)].reshape(D, TB)
            x_v[b] = (x2 + jnp.tile(2.0 * mod_v[_span(5, D), :], (1, NL)) * _block(_strassen(outer))).astype(BF)
            cp_out(b).start()

        for cp in cp_w:
            cp.wait()
        lax.fori_loop(0, NF, gate_up, None)
        lax.fori_loop(0, NB, down, None)
        for b in range(NB):
            cp_out(b).wait()

    scratch = [pltpu.VMEM(shape, F32) for shape in (
        (2 * F // LANES, S // 2 + SUB, LANES), (NB * GB, GR, TB), (NB * GB, GR, TB), (NB * GB, HG, VR, TB),
        (KC, TB), (VR, TB), (NB, H, TB), (1, S // 2, FW), (1, S // 2, FW), (7, S // 2, 3 * LANES), (6 * D, LANES))]
    scratch += [pltpu.VMEM(shape, BF) for shape in (
        (NB, D, TB), (NF, D, FW), (NF, D, FW), (NF, D, FW), (D, D), (D, D), (D, 2 * D), (D, 4 * D))]
    scratch += [pltpu.VMEM(shape, F32) for shape in ((DP + 2 * SUB, D), (D, D))]
    scratch += [pltpu.VMEM(shape, BF) for shape in ((NF, 7, HD // 2, 7 * LANES), (DH, D), (DH, D), (1, D))]
    return pl.pallas_call(
        kernel,
        out_shape=jax.ShapeDtypeStruct((D, S), BF),
        in_specs=[pl.BlockSpec(memory_space=pl.ANY)] * 10,
        out_specs=pl.BlockSpec(memory_space=pl.ANY),
        scratch_shapes=scratch + [pltpu.SemaphoreType.DMA((8 + NB,))],
        compiler_params=pltpu.CompilerParams(vmem_limit_bytes=124 * 2 ** 20),
        name="adaln_mqa_swiglu",
    )


@jax.jit
def pallas_adaLN_cond__grouped_kv_mqa__swiglu_ffn__prompt_kernel(
    A_x: jax.Array,
    A_wq: jax.Array,
    A_wk: jax.Array,
    A_wv: jax.Array,
    A_wo: jax.Array,
    B_x: jax.Array,
    B_w_gate: jax.Array,
    B_w_up: jax.Array,
    B_w_down: jax.Array,
    c: jax.Array,
    w_mod: jax.Array,
):
    del B_x
    _, S, D = A_x.shape
    out = _build(S, D, B_w_gate.shape[1])(
        A_x.reshape(S, D).T, A_wq, A_wk.T, A_wv.T, A_wo, B_w_gate, B_w_up, B_w_down.T, c, w_mod)
    return out.T.reshape(1, S, D)
```

```python
import math

import jax
import jax.numpy as jnp
from jax import lax
import jax.experimental.pallas as pl
import jax.experimental.pallas.tpu as pltpu

BF = jnp.bfloat16
F32 = jnp.float32
LANES = 128
SUB = 8
N_HEADS = 32
EPS = 1e-5
ROW_SUM_MIN = 2.0 ** -30
ROW_SUM_MAX = 2.0 ** 100

_STRASSEN = (
    (((1, 1, 1), (1, 0, 0)), ((1, 1, 1), (1, 0, 0)), ((1, 0, 0), (1, 1, 1))),
    (((1, 1, 0), (1, 1, 1)), ((1, 0, 0),), ((1, 1, 0), (-1, 1, 1))),
    (((1, 0, 0),), ((1, 0, 1), (-1, 1, 1)), ((1, 0, 1), (1, 1, 1))),
    (((1, 1, 1),), ((1, 1, 0), (-1, 0, 0)), ((1, 0, 0), (1, 1, 0))),
    (((1, 0, 1), (1, 0, 0)), ((1, 1, 1),), ((-1, 0, 0), (1, 0, 1))),
    (((1, 1, 0), (-1, 0, 0)), ((1, 0, 0), (1, 0, 1)), ((1, 1, 1),)),
    (((1, 0, 1), (-1, 1, 1)), ((1, 1, 0), (1, 1, 1)), ((1, 0, 0),)),
)
_ORDER = (1, 0, 3, 4, 6, 2, 5)
_INNER_ORDER = (1, 3, 4, 2, 0, 6, 5)


def _strassen(prod, mirror=False, order=_ORDER):
    c = {}
    for j in order:
        a, b, outs = _STRASSEN[j]
        m = prod(j, a, tuple((s, k, n ^ mirror) for s, k, n in b))
        for s, r, n in outs:
            key = r, n ^ mirror
            c[key] = (1, _signed_sum([(s, m), c[key]])) if key in c else (s, m)
    return [[c[r, n][1] for n in range(2)] for r in range(2)]


def _strassen_wide(prod):
    x1 = prod(((1, 0, 0), (1, 1, 1)), None, ((1, 0, 0), (1, 1, 1)), ())
    p4 = prod(((1, 1, 1),), ((1, 0, 0),), ((1, 1, 0), (-1, 0, 0)), ((1, 0, 0), (-1, 1, 0)))
    p5 = prod(((1, 0, 0), (1, 0, 1)), None, ((1, 1, 1),), ((-1, 1, 0),))
    c11 = prod(((1, 0, 1), (-1, 1, 1)), ((1, 0, 2),), ((1, 1, 0), (1, 1, 1)), ((1, 2, 0),)) + (p4 - p5 + x1)
    p2 = prod(((1, 1, 0), (1, 1, 1)), None, ((1, 0, 0),), ((-1, 0, 1),))
    p3 = prod(((1, 0, 0),), ((1, 1, 1),), ((1, 0, 1), (-1, 1, 1)), ((1, 1, 1), (-1, 0, 1)))
    c22 = prod(((1, 1, 0), (-1, 0, 0)), ((1, 1, 2),), ((1, 0, 0), (1, 0, 1)), ((1, 2, 1),)) + (p3 + (x1 - p2))
    y1 = prod(((1, 0, 0), (1, 1, 1)), None, (), ((1, 0, 1), (1, 1, 0)))
    c12 = prod(((1, 0, 2),), ((1, 0, 1), (-1, 1, 1)), ((1, 2, 1),), ((1, 1, 0), (1, 1, 1))) + (y1 + (p3 + p5))
    c21 = prod(((1, 1, 2),), ((1, 1, 0), (-1, 0, 0)), ((1, 2, 0),), ((1, 0, 0), (1, 0, 1))) + (y1 + (p2 + p4))
    return [[c11, c12], [c21, c22]]


def _left_sums(a11, a12, a21, a22):
    return a11 + a22, a21 + a22, a11, a22, a11 + a12, a21 - a11, a12 - a22


def _signed_sum(terms):
    (sign, out), *rest = sorted(terms, key=lambda t: -t[0])
    if rest or sign < 0:
        out = out.astype(F32) if sign > 0 else -out.astype(F32)
    for sign, t in rest:
        out = out + t.astype(F32) if sign > 0 else out - t.astype(F32)
    return out


def _block(c):
    return jnp.concatenate([jnp.concatenate(row, axis=1) for row in c], axis=0)


def _dot(a, b, trans_b=False):
    return lax.dot_general(a, b, (((1,), (1 if trans_b else 0,)), ((), ())), preferred_element_type=F32)


def _span(i, n):
    return slice(i * n, (i + 1) * n)


def _lane(l):
    return _span(l, LANES)


def _zeros_from(i):
    count = [0]

    def zero():
        count[0] += 1
        return (i + count[0]) >> 16

    return zero


def _shifted(x, n, rows):
    above, below = [[jnp.zeros((m, x.shape[1]), F32)] if m else [] for m in (n, rows - n - x.shape[0])]
    return jnp.concatenate(above + [x] + below, axis=0)


def _build(S, D, F):
    H = N_HEADS
    DH = D // H
    HH = DH // 2
    TB = 512
    NL = TB // LANES
    NB = S // TB
    HG = 4
    GR = HG * DH
    GB = H // HG
    VR = 24
    KC = LANES
    NC = S // KC
    G = KC // SUB
    NV = 3
    POS = ((15, 8, 3), (6, 12, 1))
    UNROLL = 2
    QSCALE = DH ** -0.5 * math.log2(math.e)
    DP = 2 * VR + D
    FW = 512
    NF = F // FW
    HB, HD, HF, QS = TB // 2, D // 2, FW // 2, S // 4
    K1 = 2 * LANES
    PACE = (0, 1, 2, 3, 4, 5, 6, 7, 8, 9, 14, 15, 16, 17, 18, 19)
    assert (D, DH) == (576, 18) and S % (2 * TB) == 0 and F % FW == 0 and 2 * NC <= 2 * F // LANES

    def norm(x, scale, shift):
        mean = jnp.sum(x, axis=0, keepdims=True) * (1.0 / D)
        xc = x - mean
        variance = jnp.sum(xc * xc, axis=0, keepdims=True) * (1.0 / D)
        return xc * lax.rsqrt(variance + EPS) * scale + shift

    def sum_row(j):
        return DH + 2 * j if DH + 2 * j < VR else 0

    def arrange(pos, groups):
        rows = dict(zip([g for g in reversed(range(G)) if g not in pos] + list(pos), groups))
        return jnp.concatenate([rows[g] for g in range(G)], axis=0)

    def kernel(x_hbm, wq_hbm, wk_hbm, wv_hbm, wo_hbm, wg_hbm, wu_hbm, wd_hbm, c_hbm, wm_hbm, out_hbm,
               act_v, q_v, t_v, o_v, p_v, pa_v, r_v, s_v, a_v, mod_v, x_v, wg_v, wu_v, wd_v,
               wq_v, wo_v, wm0_v, wm1_v, wp_v, wot_v, u_v, wk_v, wv_v, c_v, sem):

        def ks_rows(n, d):
            return _span(n * HH + d, SUB)

        def kb_rows(d):
            return _span(7 * HH + d, SUB)

        def vt_rows(j, t):
            return pl.ds((7 * HH + DH) * SUB + (2 * j + t) * VR, VR)

        cp_c, cp_k, cp_v, cp_q, cp_o, cp_m0, cp_m1, *cp_x = [
            pltpu.make_async_copy(src, dst, sem.at[n]) for n, (src, dst) in enumerate(
                [(c_hbm, c_v), (wk_hbm, wk_v), (wv_hbm, wv_v), (wq_hbm, wq_v), (wo_hbm, wo_v),
                 (wm_hbm.at[:, pl.ds(0, 2 * D)], wm0_v), (wm_hbm.at[:, pl.ds(2 * D, 4 * D)], wm1_v)]
                + [(x_hbm.at[:, pl.ds(b * TB, TB)], x_v.at[b]) for b in range(NB)])]
        cp_w = [pltpu.make_async_copy(src.at[:, pl.ds(i * FW, FW)], dst.at[i], sem.at[7 + NB + n * NF + i])
                for n, (src, dst) in enumerate(((wg_hbm, wg_v), (wu_hbm, wu_v), (wd_hbm, wd_v))) for i in range(NF)]

        def cp_out(b):
            return pltpu.make_async_copy(x_v.at[b], out_hbm.at[:, pl.ds(b * TB, TB)], sem.at[7 + b])

        def modulation(w, first):
            m = _dot(wp_v[DP:DP + SUB, :], w)
            mod_v[first:first + w.shape[1], :] = jnp.tile(m, (LANES // SUB, 1)).T

        for cp in [cp_m0, cp_c, cp_k, cp_v, cp_x[0], cp_q] + cp_x[1:]:
            cp.start()
        p_v[...] = jnp.zeros_like(p_v)
        pa_v[...] = jnp.zeros_like(pa_v)
        cp_m0.wait()
        cp_c.wait()
        cc = c_v[...].astype(F32)
        wp_v[DP:DP + SUB, :] = jnp.broadcast_to(cc * jax.nn.sigmoid(cc), (SUB, D))
        modulation(wm0_v[...], 0)
        mod_v[_span(1, D), :] += 1.0
        cp_k.wait()
        cp_v.wait()
        cp_x[0].wait()
        wp_v[0:2 * VR, :] = jnp.concatenate([_shifted(w[...].astype(F32), 0, VR) for w in (wk_v, wv_v)], axis=0)

        def norm1(b, l):
            return norm(x_v[b, :, _lane(l)].astype(F32), mod_v[_span(1, D), :], mod_v[_span(0, D), :])

        def put_kv(c, kt, vt):
            kk = jnp.concatenate([_shifted(kt, 2 * j, LANES // HG) for j in range(HG)], axis=0).T
            kk = jnp.concatenate(
                [kk[_span(g, SUB)] for g in list(reversed(range(G - NV))) + list(range(G - NV, G))], axis=0)
            row = lax.broadcasted_iota(jnp.int32, (VR, KC), 0)
            for t, pos in enumerate(POS):
                free = [g for g in range(G) if g not in pos]
                src = [G - NV + pos.index(g) if g in pos else free.index(g) for g in range(G)]
                cuts = [g for g in range(G) if g == 0 or src[g] != src[g - 1] + 1] + [G]
                v = jnp.concatenate([vt[:, src[a] * SUB:(src[a] + e - a) * SUB] for a, e in zip(cuts, cuts[1:])],
                                    axis=1)
                for j in range(HG):
                    act_v[c, vt_rows(j, t), :] = jnp.where(row == sum_row(j), 1.0, _shifted(v[:DH], 2 * j, VR))
            for j in range(HG):
                act_v[NC + c, _span(j, KC), 0:VR] = kk[:, j * (LANES // HG):j * (LANES // HG) + VR]

            def spread(g, d):
                return jnp.broadcast_to(kk[_span(g, SUB), d:d + 1], (SUB, LANES))

            for d in range(HH):
                a11, a12, a21, a22 = [spread(G - NV + g, d + k) for g in range(2) for k in (0, HH)]
                s1 = a21 + a22
                s2 = s1 - a11
                for n, a in enumerate((a11, a12, a12 - s2, a22, s1, s2, a11 - a21)):
                    act_v[c, ks_rows(n, d), :] = a
            for d in range(DH):
                act_v[c, kb_rows(d), :] = spread(G - 1, d)

        def put_q(b, l, left, right):
            low = lax.broadcasted_iota(jnp.int32, (GR, LANES), 0) % DH < HH
            for g in range(GB):
                qa, qb = left[_span(g, GR)], right[_span(g, GR)]
                t13 = qb - jnp.where(low, qa, _shifted(qb[:GR - HH], HH, GR))
                t2 = qb - _shifted(t13[:GR - HH], HH, GR)
                q_v[b * GB + g, :, _lane(l)] = qa
                q_v[b * GB + g, :, _lane(l + NL // 2)] = qb
                t_v[b * GB + g, :, _lane(l)] = t13
                t_v[b * GB + g, :, _lane(l + NL // 2)] = jnp.where(low, _shifted(t2[HH:], 0, GR), qa - t2)

        tiles = [(b, l + t) for b in range(NB) for l in range(NL // 2) for t in (0, NL // 2)]
        early = [norm1(*t) for t in tiles[:2]]
        cp_q.wait()
        wp_v[2 * VR:DP, :] = wq_v[...].T.astype(F32)
        prev = centre = left = None
        for n in range(len(tiles) + 1):
            if n < len(tiles):
                if n == NL:
                    for cp in cp_x[1:]:
                        cp.wait()
                    for cp in [cp_m1, cp_o] + cp_w:
                        cp.start()
                r = _dot(wp_v[0:DP, :], early[n] if n < len(early) else norm1(*tiles[n]))
            if n:
                b, l = tiles[n - 1]
                if n == 1:
                    centre = jnp.mean(prev[0:DH], axis=1, keepdims=True)
                put_kv(b * NL + l, prev[0:DH] - centre, prev[VR:2 * VR])
                if n % 2:
                    left = prev[2 * VR:] * QSCALE
                else:
                    put_q(b, l - NL // 2, left, prev[2 * VR:] * QSCALE)
            prev = r

        push_order = [(l + NL // 2) % NL for l in range(NL)]

        def finish(g):
            for l in push_order:
                o_v[g, HG - 1, :, _lane(l)] = (
                    _dot(act_v[NC - 1, vt_rows(HG - 1, l // (NL // 2)), :], p_v[:, _lane(l)]) + pa_v[:, _lane(l)])

        def vector_scores(g0, g1, j, c):
            def chain(keys, ref, g, k, l, acc=None):
                for d, key in enumerate(keys):
                    t = key * ref[g, pl.ds(j * DH + k + d, 1), _lane(l)]
                    acc = t if acc is None else acc + t
                return acc

            ks = [[act_v[c, ks_rows(n, d), :] for d in range(HH)] for n in range(7)]
            kb = [act_v[c, kb_rows(d), :] for d in range(DH)]
            out = [None] * NL
            for la in range(NL // 2):
                lb = la + NL // 2
                p1 = chain(ks[0], q_v, g0, 0, la)
                c11 = chain(ks[1], q_v, g0, HH, la, p1)
                u2 = chain(ks[5], t_v, g0, 0, lb, p1)
                u3 = chain(ks[6], t_v, g0, HH, la, u2)
                p5 = chain(ks[4], t_v, g0, 0, la)
                out[lb] = [chain(ks[2], q_v, g0, HH, lb, u2 + p5), u3 + p5]
                out[la] = [c11, chain(ks[3], t_v, g0, HH, lb, u3)]
            for l in range(NL):
                out[l].append(chain(kb[:HH], q_v, g1, 0, l) + chain(kb[HH:], q_v, g1, HH, l))
            return out

        def attend_centred(i, _):
            zero = _zeros_from(i)

            def mxu_scores(g, j, c):
                return jnp.exp2(_dot(act_v[NC + c, j * KC:(j + 1) * KC - NV * SUB, 0:VR],
                                     q_v[g, 2 * SUB * j:2 * SUB * j + VR, :]))

            def weights(g, j, c, e):
                fresh = _zeros_from(i + 2 * c)
                extra = vector_scores(g + fresh(), g + fresh(), j, c)
                return [arrange(POS[l // (NL // 2)], [e[_span(x, SUB), _lane(l)] for x in range(G - NV)]
                                + [jnp.exp2(v) for v in extra[l]]) for l in range(NL)]

            def accumulate(j, c, p, acc):
                new = {l: _dot(act_v[c, vt_rows(j, l // (NL // 2)), :], p[l]) + acc[l] for l in push_order}
                return [new[l] for l in range(NL)]

            last = None
            for n in range(UNROLL * HG):
                g, j, base = i * UNROLL + n // HG, n % HG, zero()
                e = mxu_scores(g, j, base)
                if last:
                    o_v[last[0], last[1]] = jnp.concatenate(accumulate(*last[1:]), axis=1)
                else:
                    finish(jnp.maximum(g - 1, 0))

                def step(c, carry):
                    e, acc = carry
                    return mxu_scores(g, j, base + c + 1), accumulate(j, base + c, weights(g, j, base + c, e), acc)

                e, acc = lax.fori_loop(0, NC - 1, step, (e, [jnp.zeros((VR, LANES), F32)] * NL), unroll=True)
                last = g, j, base + NC - 1, weights(g, j, base + NC - 1, e), acc
            p_v[...] = jnp.concatenate(last[3], axis=1)
            pa_v[...] = jnp.concatenate(last[4], axis=1)

        def attend_row_max(u, _):
            g, j = u // HG, u % HG
            q = q_v[g, pl.ds(pl.multiple_of(2 * SUB * j, SUB), VR), :]
            m = acc = None
            for c in range(NC):
                s = _dot(act_v[NC + c, pl.ds(pl.multiple_of(j * KC, KC), KC), 0:VR], q)
                s_v[c] = s
                t = jnp.max(s, axis=0, keepdims=True)
                m = jnp.maximum(m, t) if c else t
            for c in range(NC):
                p = jnp.exp2(s_v[c + (u >> 16)] - m)
                a = _dot(act_v[c, vt_rows(j, 0), :], arrange(POS[0], [p[_span(x, SUB)] for x in range(G)]))
                acc = a + acc if c else a
            o_v[g, j] = acc

        lax.fori_loop(0, NB * GB // UNROLL, attend_centred, None)

        def heads(b, l, checks):
            row = lax.broadcasted_iota(jnp.int32, (SUB, LANES), 0)
            for h0 in range(0, H, SUB):
                total = None
                for h in range(h0, h0 + SUB):
                    t = o_v[b * GB + h // HG, h % HG, pl.ds(sum_row(h % HG), 1), _lane(l)]
                    total = t if total is None else jnp.where(row == h - h0, t, total)
                checks.append((total >= ROW_SUM_MIN) & (total <= ROW_SUM_MAX))
                r_v[b, h0:h0 + SUB, _lane(l)] = 1.0 / total
            out = []
            for h in range(H):
                o = o_v[b * GB + h // HG, h % HG, :, _lane(l)] * r_v[b, pl.ds(h, 1), _lane(l)]
                top = jnp.where(row < 2 * (h % HG), out.pop(), o[:SUB]) if h % HG else o[:SUB]
                out += [top, o[SUB:2 * SUB], o[2 * SUB:]]
            return jnp.concatenate(out, axis=0)

        def project_out(b, l, checks):
            h2 = []
            for t in (l, l + NL // 2):
                o = heads(b, t, checks)
                attn = None
                for k in range(0, D, LANES):
                    a = _dot(wot_v[:, k:min(k + LANES, D)], o[k:k + LANES])
                    attn = a + attn if k else a
                checks.append(jnp.abs(attn[:SUB]) < jnp.inf)
                x2 = x_v[b, :, _lane(t)].astype(F32) + mod_v[_span(2, D), :] * attn
                t_v[_span(b, GB), :, _lane(t)] = x2.reshape(GB, GR, LANES)
                h = norm(x2, mod_v[_span(4, D), :], mod_v[_span(3, D), :])
                h2.append(jnp.concatenate([h, h[2 * K1:]], axis=0).T)
            rows = _span(b * (NL // 2) + l, LANES)
            for j, a in enumerate(_left_sums(*[h[:, k:k + K1] for h in h2 for k in (0, K1)])):
                a_v[j, rows, 0:K1] = a
            r1, r2 = [h[:, 2 * K1:] for h in h2]
            for j, a in ((0, r2), (3, r2), (4, r1), (6, r1 - r2)):
                a_v[j, rows, K1:] = a

        cp_m1.wait()
        cp_o.wait()
        finish(NB * GB - 1)
        wot_v[...] = wo_v[...].T.astype(F32)
        modulation(wm1_v[...], 2 * D)
        mod_v[_span(3, D), :] *= 0.5
        mod_v[_span(4, D), :] = 0.5 * mod_v[_span(4, D), :] + 0.5
        mod_v[_span(5, D), :] *= 2.0

        def attempt(state):
            @pl.when(state[0] == 1)
            def _():
                lax.fori_loop(0, NB * H, attend_row_max, None)

            checks = []
            for b in range(NB):
                for l in range(NL // 2):
                    project_out(b, l, checks)
            good = jnp.ones((SUB, LANES), F32)
            for ok in checks:
                good = jnp.where(ok, good, 0.0)
            return state[0] + 1, jnp.min(good).astype(jnp.int32)

        lax.while_loop(lambda state: (state[0] < 2) & (state[1] == 0), attempt, (0, 0))

        def gate_up(i, _):
            zero = _zeros_from(i)
            passes = []

            def outer(j, a, b):
                rest = [t for t in b if t[1] == 1] if b[0][1] == 1 else []

                def left(z, terms):
                    return _signed_sum([(s, a_v[z, _span(m, QS), _lane(k)]) for s, m, k in terms])

                def right(terms, first, rows):
                    z = i + zero()
                    return jnp.concatenate([_signed_sum([
                        (s * ss, w[z, pl.ds(k * K1 + kk * LANES + first * (kk < 2), rows), _lane(2 * n + nn)])
                        for ss, kk, nn in terms for s, k, n in (b if kk < 2 else rest)]) for w in (wg_v, wu_v)], axis=1)

                def inner(jj, aa, bb):
                    lhs, rhs = left(j + zero(), aa), right(bb, 0, LANES)
                    if j == jj == _ORDER[-1]:
                        return jnp.concatenate([_dot(lhs[_span(m, QS // 2)], rhs) for m in range(2)], axis=0)
                    passes.append(_dot(lhs, rhs))
                    return passes[-1]

                def wide(a_low, a_high, b_low, b_high):
                    z = j + zero()
                    half = LANES // 2
                    lhs = left(z, a_low)
                    if a_high:
                        lhs = jnp.where(lax.broadcasted_iota(jnp.int32, lhs.shape, 1) < half, lhs, left(z, a_high))
                    rhs = [right(t, first, half).astype(F32) if t else jnp.zeros((half, HF), F32)
                           for t, first in ((b_low, 0), (b_high, half))]
                    passes.append(_dot(lhs, jnp.concatenate(rhs, axis=0)))
                    return passes[-1]

                return _block(_strassen_wide(wide) if rest else _strassen(inner, j == 5, _INNER_ORDER))

            for m, row in enumerate(_strassen(outer)):
                row = jnp.concatenate(row, axis=1)
                for l in range(FW // LANES):
                    t, up = row[:, _lane(2 * l)], row[:, _lane(2 * l + 1)]
                    silu = t + t * jnp.tanh(t)
                    act_v[(m * NF + i) * (FW // LANES) + l, 0:S // 2, :] = silu * up

            always = lax.broadcasted_iota(jnp.int32, (2 * SUB, HF), 0) >= zero()
            jobs = [(j, r) for j in range(7) for r in range(0, HD // 2, SUB)]
            slab = [i + zero() for _ in range(7)]
            for n, (j, r) in enumerate(jobs):
                w = _signed_sum([
                    (s, jnp.concatenate([wd_v[slab[j], pl.ds(m * HD + o + r, SUB), _span(k, HF)].astype(F32)
                                         for o in (0, HD // 2)], axis=0)) for s, m, k in _STRASSEN[j][0]])
                when, row = divmod(n * len(PACE) * (QS // SUB) // len(jobs), QS // SUB)
                w = jnp.where(always, w, jnp.tile(passes[2 * PACE[when] + 1][_span(row, SUB)], (2, 1)))
                sums = _left_sums(*[w[_span(m, SUB), _lane(k)] for m in range(2) for k in range(2)])
                u_v[i, j, r:r + SUB, :] = jnp.concatenate(sums, axis=1).astype(BF)

        def down(b, _):
            zero = _zeros_from(b)

            def outer(j, _, terms):
                def inner(jj, _, sub):
                    r0 = pl.multiple_of((b + zero()) * HB, HB)
                    acc = None
                    for i in range(NF):
                        rhs = _signed_sum([
                            (s * ss, act_v[(n * NF + i) * (FW // LANES) + 2 * k + kk, pl.ds(r0 + nn * LANES, LANES), :])
                            for ss, kk, nn in sub for s, k, n in terms])
                        lhs = u_v[i, j, :, _lane(jj)]
                        if j == jj == _ORDER[-1] and i == NF - 1:
                            r = jnp.concatenate([_dot(lhs[_span(m, HD // 6)], rhs.astype(BF), True)
                                                 for m in range(3)], axis=0)
                        else:
                            r = _dot(lhs, rhs.astype(BF), True)
                        acc = r + acc if i else r
                    return acc

                return _block(_strassen(inner, j in (1, 4, 5, 6), _INNER_ORDER))

            x2 = t_v[pl.ds(b * GB, GB)].reshape(D, TB)
            x_v[b] = (x2 + jnp.tile(mod_v[_span(5, D), :], (1, NL)) * _block(_strassen(outer))).astype(BF)
            cp_out(b).start()

        for cp in cp_w:
            cp.wait()
        lax.fori_loop(0, NF, gate_up, None)
        lax.fori_loop(0, NB, down, None)
        for b in range(NB):
            cp_out(b).wait()

    scratch = [pltpu.VMEM(shape, F32) for shape in (
        (2 * F // LANES, S // 2 + SUB, LANES), (NB * GB, GR, TB), (NB * GB, GR, TB), (NB * GB, HG, VR, TB),
        (KC, TB), (VR, TB), (NB, H, TB), (NC, KC, TB), (7, S // 2, 3 * LANES), (6 * D, LANES))]
    scratch += [pltpu.VMEM(shape, BF) for shape in (
        (NB, D, TB), (NF, D, FW), (NF, D, FW), (NF, D, FW), (D, D), (D, D), (D, 2 * D), (D, 4 * D))]
    scratch += [pltpu.VMEM(shape, F32) for shape in ((DP + 2 * SUB, D), (D, D))]
    scratch += [pltpu.VMEM(shape, BF) for shape in ((NF, 7, HD // 2, 7 * LANES), (DH, D), (DH, D), (1, D))]
    return pl.pallas_call(
        kernel,
        out_shape=jax.ShapeDtypeStruct((D, S), BF),
        in_specs=[pl.BlockSpec(memory_space=pl.ANY)] * 10,
        out_specs=pl.BlockSpec(memory_space=pl.ANY),
        scratch_shapes=scratch + [pltpu.SemaphoreType.DMA((7 + NB + 3 * NF,))],
        compiler_params=pltpu.CompilerParams(vmem_limit_bytes=124 * 2 ** 20),
        name="adaln_mqa_swiglu",
    )


@jax.jit
def pallas_adaLN_cond__grouped_kv_mqa__swiglu_ffn__prompt_kernel(
    A_x: jax.Array,
    A_wq: jax.Array,
    A_wk: jax.Array,
    A_wv: jax.Array,
    A_wo: jax.Array,
    B_x: jax.Array,
    B_w_gate: jax.Array,
    B_w_up: jax.Array,
    B_w_down: jax.Array,
    c: jax.Array,
    w_mod: jax.Array,
):
    del B_x
    _, S, D = A_x.shape
    out = _build(S, D, B_w_gate.shape[1])(
        A_x.reshape(S, D).T, A_wq, A_wk.T, A_wv.T, A_wo, B_w_gate, B_w_up, B_w_down.T, c, w_mod)
    return out.T.reshape(1, S, D)
```
